```python
import os as _os
_os.environ.setdefault("JAX_PLATFORMS", "cpu")
import jax
import jax.numpy as jnp

def _softmax(x, axis=-1):
    return jax.nn.softmax(x, axis=axis)
def _gelu(x):
    return jax.nn.gelu(x, approximate=True)
def _silu(x):
    return jax.nn.silu(x)
def _sigmoid(x):
    return jax.nn.sigmoid(x)
def _layernorm(x, axis=-1, eps=1e-5):
    m = jnp.mean(x, axis=axis, keepdims=True)
    v = jnp.var(x, axis=axis, keepdims=True)
    return (x - m) / jnp.sqrt(v + eps)
def _scatter_add(tgt, idx, src, axis=0):
    return tgt.at[idx].add(src)
def _segment_sum(src, seg, n):
    return jax.ops.segment_sum(src, seg, n)
class _Rng:
    def __init__(self, key):
        self._k = key
    def _next(self):
        self._k, sub = jax.random.split(self._k)
        return sub
    def normal(self, shape):
        return jax.random.normal(self._next(), shape, dtype=jnp.bfloat16)
    def randint(self, lo, hi, shape):
        return jax.random.randint(self._next(), shape, lo, hi, dtype=jnp.int32)
    def uniform(self, shape, lo=0.0, hi=1.0):
        return jax.random.uniform(self._next(), shape, jnp.bfloat16, lo, hi)
    def permutation(self, n):
        return jax.random.permutation(self._next(), n)


kernel_name = 'recurrent_scan__ssm_conv_s4__mixer_s_mlp__prompt'

def setup_inputs():
    _rng = _Rng(jax.random.key(int.from_bytes(__import__("os").urandom(4), "little")))
    _w = (lambda a: (lambda t: t.astype(jnp.bfloat16) if jnp.issubdtype(t.dtype, jnp.floating) else t)(jnp.asarray(a)))
    def _A_setup():
        B, L, D, N = 1, 2048, 512, 128
        A_re = -jnp.exp((lambda *s: _rng.normal(s) * 0.1)(D, N))
        A_im = jnp.pi * (lambda *s: _rng.normal(s) * 0.1)(D, N)
        B_re = (lambda *s: _rng.normal(s) * 0.1)(D, N)
        B_im = (lambda *s: _rng.normal(s) * 0.1)(D, N)
        C_re = (lambda *s: _rng.normal(s) * 0.1)(D, N)
        C_im = (lambda *s: _rng.normal(s) * 0.1)(D, N)
        log_dt = (lambda *s: _rng.normal(s) * 0.1)(D) * 0.5 - 4.0
        Dskip = (lambda *s: _rng.normal(s) * 0.05)(D)
        return {
            "u": _w((lambda *s: _rng.normal(s) * 0.05)(B, L, D)),
            "A_re": _w(A_re),
            "A_im": _w(A_im),
            "B_re": _w(B_re),
            "B_im": _w(B_im),
            "C_re": _w(C_re),
            "C_im": _w(C_im),
            "log_dt": _w(log_dt),
            "Dskip": _w(Dskip),
        }
    _A_in = _A_setup()

    def _B_setup():
        B, S, D, F = 1, 2048, 512, 1376
        return {
            "x":  _w((lambda *s: _rng.normal(s) * 0.05)(B, S, D)),
            "w1": _w((lambda *s: _rng.normal(s) * 0.8)(D, D) * (D ** -0.5)),
            "w2": _w((lambda *s: _rng.normal(s) * 0.8)(D, D) * (D ** -0.5)),
            "w3": _w((lambda *s: _rng.normal(s) * 0.8)(D, F) * (D ** -0.5)),
            "w4": _w((lambda *s: _rng.normal(s) * 0.8)(F, D) * (F ** -0.5)),
        }
    _B_in = _B_setup()

    return {
        "A_u": _A_in["u"],
        "A_A_re": _A_in["A_re"],
        "A_A_im": _A_in["A_im"],
        "A_B_re": _A_in["B_re"],
        "A_B_im": _A_in["B_im"],
        "A_C_re": _A_in["C_re"],
        "A_C_im": _A_in["C_im"],
        "A_log_dt": _A_in["log_dt"],
        "A_Dskip": _A_in["Dskip"],
        "B_x": _B_in["x"],
        "B_w1": _B_in["w1"],
        "B_w2": _B_in["w2"],
        "B_w3": _B_in["w3"],
        "B_w4": _B_in["w4"],
    }

def reference(A_u, A_A_re, A_A_im, A_B_re, A_B_im, A_C_re, A_C_im, A_log_dt, A_Dskip, B_x, B_w1, B_w2, B_w3, B_w4):
    def _A_ref(u, A_re, A_im, B_re, B_im, C_re, C_im, log_dt, Dskip):
        Bsz, L, D = u.shape
        dt = jnp.exp(log_dt)[:, None]
        A = A_re + 1j * A_im
        Bc = B_re + 1j * B_im
        Cc = C_re + 1j * C_im
        logdA = dt * A
        dB = dt * Bc
        l = (lambda x, dt: x.astype(dt))(jnp.arange(L), A_re.dtype)
        P = jnp.exp(logdA[:, :, None] * l[None, None, :])
        K = jnp.einsum("dn,dnl,dn->dl", Cc, P, dB).real
        L2 = 2 * L
        Kp = jnp.pad(K, ((0, 0), (0, L)))
        up = (lambda x, *d: x.transpose(*d))(u, 0, 2, 1)
        up = jnp.pad(up, ((0, 0), (0, 0), (0, L)))
        Kf = (lambda x, axes=(-2,-1): jnp.fft.rfft2(x.astype(jnp.float32), axes=axes))(Kp[:, None, :], axes=(-2, -1))
        Uf = (lambda x, axes=(-2,-1): jnp.fft.rfft2(x.astype(jnp.float32), axes=axes))(up[:, :, None, :], axes=(-2, -1))
        Yf = Uf * Kf[None, :, :, :]
        y = (lambda x, s, axes=(-2,-1): jnp.fft.irfft2(x, s=s, axes=axes).astype(jnp.bfloat16))(Yf, (1, L2), axes=(-2, -1))[:, :, 0, :L]
        y = (lambda x, *d: x.transpose(*d))(y, 0, 2, 1) + u * Dskip[None, None, :]
        return y

    def _B_ref(x, w1, w2, w3, w4):
        B, S, D = x.shape
        h = _gelu(_layernorm(x, axis=-1) @ w1)
        c = D // 4
        g0 = jnp.pad(h[:, :, 0*c:1*c], ((0, 0), (1, 0), (0, 0)))[:, :S, :]
        g1 = jnp.pad(h[:, :, 1*c:2*c], ((0, 0), (0, 1), (0, 0)))[:, 1:, :]
        g2 = jnp.pad(h[:, :, 2*c:3*c], ((0, 0), (2, 0), (0, 0)))[:, :S, :]
        g3 = jnp.pad(h[:, :, 3*c:   ], ((0, 0), (0, 2), (0, 0)))[:, 2:, :]
        hs = jnp.concatenate([g0, g1, g2, g3], axis=-1) @ w2
        x1 = x + hs
        h2 = _gelu(_layernorm(x1, axis=-1) @ w3) @ w4
        return x1 + h2

    x = A_u
    xn = _layernorm(x, axis=-1)
    s = _A_ref(xn, A_A_re, A_A_im, A_B_re, A_B_im, A_C_re, A_C_im, A_log_dt, A_Dskip)
    g = _silu(_B_ref(xn, B_w1, B_w2, B_w3, B_w4))
    return x + s * g
```

```python
import itertools
import ml_dtypes
import numpy as np
import jax
import jax.numpy as jnp
import jax.experimental.pallas as pl
import jax.experimental.pallas.tpu as pltpu

L, D, N, F = 2048, 512, 128, 1376
Q = 128
NB = L // Q
TS = D + 1
CH = D // NB
XS = NB + 1
SCHED = (3,) * 10 + (2, 0)
f32, bf16 = jnp.float32, jnp.bfloat16


def _constants():
    fr = np.concatenate([np.arange(0, Q, 2), np.arange(1, Q, 2)]).astype(np.float64)
    t = np.arange(Q, dtype=np.float64)
    ph = 2 * np.pi * (fr[:, None] + 0.5) * t[None, :] / (2 * Q)

    def rows(re, im):
        return np.stack([re.reshape(Q // 8, 8, -1), im.reshape(Q // 8, 8, -1)], 1).reshape(2 * Q, -1)

    fwd = rows(np.cos(ph), -np.sin(ph))
    mats = []
    for k in (0, 2, 4, 8):
        lo = (k * Q + t).astype(np.float32).astype(ml_dtypes.bfloat16).astype(np.int64) - k * Q
        lane = np.where(lo == Q, Q - 1, lo)
        sel = np.zeros((Q, Q))
        sel[np.arange(Q), lane] = 1.0
        mats.append(fwd @ sel[:, _il(Q)])
    mats.append(fwd)
    inv = (fwd / Q).T
    return (np.stack(mats).astype(ml_dtypes.bfloat16), np.ascontiguousarray(inv).astype(ml_dtypes.bfloat16))


def _cmul(a, b):
    return a[0] * b[0] - a[1] * b[1], a[0] * b[1] + a[1] * b[0]


def _csq(a):
    t = a[0] * a[1]
    return a[0] * a[0] - a[1] * a[1], t + t


def _cmulc(a, b):
    return a[0] * b[0] + a[1] * b[1], a[1] * b[0] - a[0] * b[1]


def _sincos(x):
    k = jnp.round(x * 0.6366197723675814)
    r = ((x - k * 1.5703125) - k * 4.837512969970703e-4) - k * 7.54978995489188e-8
    r2 = r * r
    s = r + r * r2 * (-1.6666654611e-1 + r2 * (8.3321608736e-3 + r2 * -1.9515295891e-4))
    c = 1.0 + r2 * (-0.5 + r2 * (4.166664568298827e-2 + r2 * (-1.388731625493765e-3 + r2 * 2.443315711809948e-5)))
    n = k.astype(jnp.int32)
    sw = (n & 1) == 1
    s, c = jnp.where(sw, c, s), jnp.where(sw, s, c)
    return jnp.where((n & 2) == 2, -s, s), jnp.where(((n + 1) & 2) == 2, -c, c)


def _pack(a, b):
    return pltpu.bitcast(pltpu.pack_elementwise([a, b], packed_dtype=bf16), bf16)


def _il(n):
    i = np.arange(n)
    return i // 16 * 16 + i % 2 * 8 + i % 16 // 2


def _ln(x):
    d = x - jnp.mean(x, -1, keepdims=True)
    return d * jax.lax.rsqrt(jnp.mean(d * d, -1, keepdims=True) + 1e-5)


def _gelu(x):
    return x * jnp.tanh(x * (0.7978845608028654 + 0.7978845608028654 * 0.044715 * (x * x))) + x


def _dot(a, b):
    return jnp.dot(a, b, preferred_element_type=f32)


def _dot_nt(a, b):
    return jax.lax.dot_general(a, b, (((1,), (1,)), ((), ())), preferred_element_type=f32)


def _body(are, aim, bre, bim, cre, cim, ldt, dsk, fwd, inv, u_h, w1_h, w2_h, w3_h, w4_h, o_h,
          u, w1, w2, w3, w4, bt, pt, zt, ke, dtc, xs, xn, hs, uh, hh, x1, l1, zz, ob, sem, osem):
    cu = [pltpu.make_async_copy(u_h.at[pl.ds(i * 512, 512)], u.at[pl.ds(i * 512, 512)], sem.at[i]) for i in range(4)]
    cw = [pltpu.make_async_copy(s, d, sem.at[4 + i])
          for i, (s, d) in enumerate(((w1_h, w1), (w2_h, w2), (w3_h, w3), (w4_h, w4)))]
    for c in (cu[0], cw[1], cw[0], cu[1], cu[2], cu[3], cw[2], cw[3]):
        c.start()

    dtr = jnp.exp(ldt[...].reshape(1, D).astype(f32)).astype(bf16).astype(f32)
    for j in range(D // 128):
        dtc[j * 128:(j + 1) * 128, :] = jnp.broadcast_to(dtr[:, j * 128:(j + 1) * 128], (128, 128)).T

    def prep(i):
        r = pl.ds(pl.multiple_of(i * CH, CH), CH)
        dt = dtc[r, :]
        mag = jnp.exp(dt * are[r, :].astype(f32))
        sn, cs = _sincos(-dt * aim[r, :].astype(f32))
        z = (mag * cs, mag * sn)
        w = _cmul((cre[r, :].astype(f32), cim[r, :].astype(f32)),
                  (dt * bre[r, :].astype(f32), dt * bim[r, :].astype(f32)))
        p2 = [z]
        for _ in range(10):
            p2.append(_csq(p2[-1]))
        b = [(jnp.ones_like(dt), jnp.zeros_like(dt)), z, p2[1], _cmul(z, p2[1]), p2[2]]
        b += [_cmul(b[m], p2[2]) for m in (1, 2, 3)]
        p = [w]
        for m in range(3):
            p += [_cmulc(v, p2[7 + m]) for v in p]
        e = _cmulc(w, _cmul(_cmul(_cmul(b[7], p2[3]), _cmul(p2[4], p2[5])), p2[6]))
        z9 = _cmul(z, p2[3])
        for c in range(2):
            for m in range(8):
                bt[c, pl.ds(m * TS + i * CH, CH), :] = b[m][c]
                pt[c, pl.ds(m * TS + i * CH, CH), :] = p[m][c]
            zt[c, r, :] = p2[3][c]
            zt[2 + c, r, :] = z9[c]
            zt[4 + c, r, :] = p2[10][c]
        ke[0, r, :] = jnp.broadcast_to(jnp.sum(e[0], -1, keepdims=True), (CH, 128))
        ke[1, r, :] = jnp.broadcast_to(
            jnp.sum(e[0] * p2[7][0] + e[1] * p2[7][1], -1, keepdims=True), (CH, 128))

    zero8 = jnp.zeros((8, 128), f32)
    for g in range(4):
        hs[g, 0:8, :] = zero8
        hs[g, L + 8:L + 16, :] = zero8

    last = jax.lax.broadcasted_iota(jnp.int32, (8, 128), 0) == 7

    def kgen(d):
        row = lambda c: jnp.broadcast_to(zt[c, pl.ds(d, 1), :], (8, 128))
        v = tuple(bt[c, pl.ds(d, 8, stride=TS), :] for c in range(2))
        z8 = (row(0), row(1))
        z8l = (jnp.where(last, row(2), z8[0]), jnp.where(last, row(3), z8[1]))
        q = []
        for j in range(8):
            if j:
                v = _cmul(v, z8)
            v2 = _cmul(v, z8l if j == 7 else z8)
            q.append([_pack(v[c], v2[c]) for c in range(2)])
            v = v2
        p0 = tuple(pt[c, pl.ds(d, 8, stride=TS), :] for c in range(2))
        p1 = _cmulc(p0, (row(4), row(5)))
        o = [_dot_nt(_pack(p0[c], p1[c]), jnp.concatenate([t[c] for t in q], 0))
             for c in range(2)]
        xs[pl.ds(d * XS, NB), :] = o[0] + o[1]

    def front(i):
        r = pl.ds(pl.multiple_of(i * Q, Q), Q)
        v = _ln(u[r, :].astype(f32)).astype(bf16)
        xn[r, :] = v
        yield
        yield
        uh[i] = _dot(fwd[4], v)
        yield
        for g in range(4):
            hs[g, pl.ds(pl.multiple_of(i * Q + 8, 8), Q), :] = _gelu(_dot(v, w1[:, g * 128:(g + 1) * 128]))
            yield

    def mid(k):
        r = pl.ds(pl.multiple_of(k * Q, Q), Q)
        g = jnp.concatenate([hs[n, pl.ds(k * Q + 8 + s, Q), :].astype(bf16)
                             for n, s in enumerate((-1, 1, -2, 2))], 1)
        y = []
        for n in range(4):
            c = slice(n * 128, (n + 1) * 128)
            y.append(xn[r, c].astype(f32) + 0.5 * _dot(g, w2[:, c]))
            yield
        y = jnp.concatenate(y, 1)
        x1[r, :] = y

    prep(0)
    cu[0].wait()
    cw[0].wait()
    cw[1].wait()
    for _ in front(0):
        pass

    def phase1(i, _):
        for k in range(1, 4):
            @pl.when(i == 4 * k - 1)
            def _():
                cu[k].wait()
        n = jnp.minimum(i + 1, NB - 1)
        d = 0
        for cnt, _unit in zip(SCHED, itertools.chain(front(n), mid(i))):
            for _ in range(cnt):
                kgen(i * CH + d)
                d += 1
        assert d == CH
        prep(n)

    jax.lax.fori_loop(0, NB, phase1, None)

    lane_last = jax.lax.broadcasted_iota(jnp.int32, (Q, 128), 1) == Q - 1

    def phase1b(k, _):
        seg = jnp.where(k < 2, 0, jnp.where(k < 4, 1, jnp.where(k < 8, 2, 3)))
        fix = jnp.logical_and(lane_last, k < 2)
        for j in range(4):
            xk = xs[pl.ds(j * 128 * XS + k % 8 * 2 + k // 8, 128, stride=XS), :]
            xk = jnp.where(fix, ke[jnp.minimum(k, 1), j * 128:(j + 1) * 128, :], xk).astype(bf16)
            cur = _dot_nt(fwd[seg], xk)
            c = slice(j * 128, (j + 1) * 128)
            hh[k, :, c] = cur

    l1[...] = _ln(x1[0:Q, :]).astype(bf16)
    jax.lax.fori_loop(0, NB, phase1b, None, unroll=8)
    cw[2].wait()
    cw[3].wait()

    def conv(t, j):
        re, im = pl.ds(pl.multiple_of(t * 16, 16), 8), pl.ds(pl.multiple_of(t * 16 + 8, 8), 8)
        c = slice(j * 128, (j + 1) * 128)
        ld = lambda ref, n: (ref[n, re, c], ref[n, im, c])
        prev = None
        sg = jnp.where(t < 8, 1.0, -1.0)
        for c0 in range(0, NB, 4):
            acc = [None] * 4
            hw = {}
            for m in range(c0 + 3, -1, -1):
                uv = ld(uh, m)
                for a in range(4):
                    k = c0 + a - m
                    if k < 0:
                        continue
                    if k not in hw:
                        hw[k] = ld(hh, k)
                    p = _cmul(uv, hw[k])
                    acc[a] = p if acc[a] is None else (acc[a][0] + p[0], acc[a][1] + p[1])
            for a in range(4):
                o = acc[a] if prev is None else (acc[a][0] - sg * prev[1], acc[a][1] + sg * prev[0])
                prev = acc[a]
                zz[c0 + a, pl.ds(pl.multiple_of(t * 16, 16), 16), c] = jnp.concatenate(o, 0).astype(bf16)
            yield

    def phase2(i, _):
        r = pl.ds(pl.multiple_of(i * Q, Q), Q)
        cv = itertools.chain(*[conv(i, j) for j in range(4)])
        v = l1[...]
        a = []
        for n in range(0, F, 128):
            a.append(_gelu(_dot_nt(v, w3[n:min(n + 128, F), :])).astype(bf16))
            next(cv)
            if n < 640:
                next(cv)
        nx = pl.ds(pl.multiple_of(jnp.minimum(i + 1, NB - 1) * Q, Q), Q)
        l1[...] = _ln(x1[nx, :]).astype(bf16)
        a = jnp.concatenate(a, 1)
        for n in range(4):
            c = slice(n * 128, (n + 1) * 128)
            b = 0.5 * x1[r, c] + 0.25 * _dot(a, w4[:, c])
            x1[r, c] = b * jnp.tanh(b) + b
        assert next(cv, None) is None

    jax.lax.fori_loop(0, NB, phase2, None)

    def out_copy(i):
        r = pl.ds(pl.multiple_of(i * 256, 256), 256)
        return pltpu.make_async_copy(ob.at[r], o_h.at[r], osem.at[i])

    dskip = dsk[...].reshape(1, D).astype(f32)

    def phase3(i, _):
        for a in range(2):
            n = 2 * i + a
            r = pl.ds(pl.multiple_of(n * Q, Q), Q)
            y = _dot(inv[...], zz[n]) + xn[r, :].astype(f32) * dskip
            ob[r, :] = (u[r, :].astype(f32) + y * x1[r, :]).astype(bf16)
        out_copy(i).start()

    jax.lax.fori_loop(0, NB // 2, phase3, None, unroll=2)
    for i in range(NB // 2):
        out_copy(i).wait()


_FWD, _INV = _constants()


@jax.jit
def pallas_recurrent_scan__ssm_conv_s4__mixer_s_mlp__prompt_kernel(
    A_u, A_A_re, A_A_im, A_B_re, A_B_im, A_C_re, A_C_im, A_log_dt, A_Dskip,
    B_x, B_w1, B_w2, B_w3, B_w4,
):
    vm = pl.BlockSpec(memory_space=pltpu.VMEM)
    hbm = pl.BlockSpec(memory_space=pl.ANY)
    V = pltpu.VMEM
    out = pl.pallas_call(
        _body,
        out_shape=jax.ShapeDtypeStruct((L, D), bf16),
        in_specs=[vm] * 10 + [hbm] * 5,
        out_specs=hbm,
        scratch_shapes=[
            V((L, D), bf16), V((D, D), bf16), V((D, D), bf16), V((F, D), bf16), V((F, D), bf16),
            V((2, 8 * TS, N), f32), V((2, 8 * TS, N), f32), V((6, D, N), f32), V((2, D, 128), f32), V((D, 128), f32),
            V((D * XS, Q), f32), V((L, D), bf16), V((4, L + 16, 128), f32),
            V((NB, 2 * Q, D), f32), V((NB, 2 * Q, D), f32),
            V((L, D), f32), V((Q, D), bf16), V((NB, 2 * Q, D), bf16), V((L, D), bf16),
            pltpu.SemaphoreType.DMA((8,)), pltpu.SemaphoreType.DMA((NB // 2,)),
        ],
        compiler_params=pltpu.CompilerParams(vmem_limit_bytes=100 << 20),
    )(A_A_re, A_A_im, A_B_re, A_B_im, A_C_re, A_C_im, A_log_dt, A_Dskip,
      jnp.asarray(_FWD), jnp.asarray(_INV), A_u.reshape(L, D), B_w1, B_w2, B_w3.T, B_w4)
    return out.reshape(1, L, D)
```
